```python
import jax
import jax.numpy as jnp

def _softmax(x, axis=-1):
    return jax.nn.softmax(x, axis=axis)
def _gelu(x):
    return jax.nn.gelu(x, approximate=True)
def _silu(x):
    return jax.nn.silu(x)
def _sigmoid(x):
    return jax.nn.sigmoid(x)
def _layernorm(x, axis=-1, eps=1e-5):
    m = jnp.mean(x, axis=axis, keepdims=True)
    v = jnp.var(x, axis=axis, keepdims=True)
    return (x - m) / jnp.sqrt(v + eps)
def _scatter_add(tgt, idx, src, axis=0):
    return tgt.at[idx].add(src)
def _segment_sum(src, seg, n):
    return jax.ops.segment_sum(src, seg, n)
class _Rng:
    def __init__(self, key):
        self._k = key
    def _next(self):
        self._k, sub = jax.random.split(self._k)
        return sub
    def normal(self, shape):
        return jax.random.normal(self._next(), shape, dtype=jnp.bfloat16)
    def randint(self, lo, hi, shape):
        return jax.random.randint(self._next(), shape, lo, hi, dtype=jnp.int32)
    def uniform(self, shape, lo=0.0, hi=1.0):
        return jax.random.uniform(self._next(), shape, jnp.bfloat16, lo, hi)
    def permutation(self, n):
        return jax.random.permutation(self._next(), n)


kernel_name = 'sequential_preLN__sliding_block_cached__moe_arch_mod__decode'

def setup_inputs():
    _rng = _Rng(jax.random.key(int.from_bytes(__import__("os").urandom(4), "little")))
    _w = (lambda a: (lambda t: t.astype(jnp.bfloat16) if jnp.issubdtype(t.dtype, jnp.floating) else t)(jnp.asarray(a)))
    def _A_setup():
        B, Sq, D = 1, 1, 640
        Hq, Hkv, Sk, Dh = 32, 32, 32768, 192
        assert Hq % Hkv == 0, (Hq, Hkv)
        return {
            "x": _w((lambda *s: _rng.normal(s) * 0.05)(B, Sq, D)),
            "k_cache": _w((lambda *s: _rng.normal(s) * 0.05)(B, Hkv, Sk, Dh)),
            "v_cache": _w((lambda *s: _rng.normal(s) * 0.05)(B, Hkv, Sk, Dh)),
            "wq": _w((lambda *s: _rng.normal(s) * 0.05)(D, Hq * Dh) * (D ** -0.5)),
            "wo": _w((lambda *s: _rng.normal(s) * 0.05)(Hq * Dh, D) * ((Hq * Dh) ** -0.5)),
        }
    _A_in = _A_setup()

    def _B_setup():
        B, S, D, F, C = 1, 1, 640, 1536, 1
        return {
            "x": _w((lambda *s: _rng.normal(s) * 0.05)(B, S, D)),
            "w_r": _w((lambda *s: _rng.normal(s) * 0.05)(D)),
            "w_gate": _w((lambda *s: _rng.normal(s) * 0.05)(D, F)),
            "w_up": _w((lambda *s: _rng.normal(s) * 0.05)(D, F)),
            "w_down": _w((lambda *s: _rng.normal(s) * 0.05)(F, D)),
        }
    _B_in = _B_setup()

    return {
        "A_x": _A_in["x"],
        "A_k_cache": _A_in["k_cache"],
        "A_v_cache": _A_in["v_cache"],
        "A_wq": _A_in["wq"],
        "A_wo": _A_in["wo"],
        "B_x": _B_in["x"],
        "B_w_r": _B_in["w_r"],
        "B_w_gate": _B_in["w_gate"],
        "B_w_up": _B_in["w_up"],
        "B_w_down": _B_in["w_down"],
    }

def reference(A_x, A_k_cache, A_v_cache, A_wq, A_wo, B_x, B_w_r, B_w_gate, B_w_up, B_w_down):
    def _A_ref(x, k_cache, v_cache, wq, wo):
        B, Sq, D = x.shape
        Hq, Dh = 32, 192
        Hkv, Sk = k_cache.shape[1], k_cache.shape[2]
        W = min(4096, max(256, Sk // 4))
        rep = Hq // Hkv
        q = (lambda x, *d: x.transpose(*d))((x @ wq).reshape(B, Sq, Hq, Dh), 0, 2, 1, 3)
        k = jnp.repeat(k_cache[:, :, Sk - W:, :], rep, axis=1)
        v = jnp.repeat(v_cache[:, :, Sk - W:, :], rep, axis=1)
        scores = jnp.einsum("bhqd,bhkd->bhqk", q, k) * (Dh ** -0.5)
        p = _softmax(scores, axis=-1)
        o = jnp.einsum("bhqk,bhkd->bhqd", p, v)
        return (lambda x, *d: x.transpose(*d))(o, 0, 2, 1, 3).reshape(B, Sq, Hq * Dh) @ wo

    def _B_ref(x, w_r, w_gate, w_up, w_down):
        B, S, D = x.shape
        C = 1
        r = x @ w_r
        idx = jnp.argsort(-r, axis=-1)[:, :C]
        idx_e = jnp.repeat(idx.reshape(B, C, 1), D, axis=2)
        x_sel = jnp.take_along_axis(x, idx_e, axis=1)
        g = _silu(x_sel @ w_gate)
        u = x_sel @ w_up
        y = (g * u) @ w_down
        r_sel = _sigmoid(jnp.take_along_axis(r, idx, axis=1))
        y = y * r_sel.reshape(B, C, 1)
        b_off = (jnp.arange(B) * S).reshape(B, 1)
        flat_idx = (idx + b_off).reshape(B * C)
        zero = (x * 0.0).reshape(B * S, D)
        upd = _scatter_add(zero, flat_idx, y.reshape(B * C, D), axis=0)
        return x + upd.reshape(B, S, D)

    x = A_x
    h = x + _A_ref(_layernorm(x, axis=-1), A_k_cache, A_v_cache, A_wq, A_wo)
    h2 = h + _B_ref(_layernorm(h, axis=-1), B_w_r, B_w_gate, B_w_up, B_w_down)
    return h2
```

```python
import functools

import jax
import jax.numpy as jnp
from jax import lax
import jax.experimental.pallas as pl
import jax.experimental.pallas.tpu as pltpu

_HQ = 32
_DH = 192
_GRP = 2 * _DH
_NT = (((1,), (1,)), ((), ()))


def _layernorm(x, eps=1e-5):
    m = jnp.mean(x, axis=-1, keepdims=True)
    d = x - m
    v = jnp.mean(d * d, axis=-1, keepdims=True)
    return d / jnp.sqrt(v + eps)


def _kernel(x_hbm, k_hbm, v_hbm, wq_hbm, wo_hbm, wr_hbm, wg_hbm, wu_hbm, wd_hbm,
            o_ref,
            x_v, wr_v, k_v, v_v, wq_v, wo_v, wg_v, wu_v, wd_v, q_v,
            sem_s, sem_k, sem_v, *, win, nbuf, nsplit):
    sk = k_hbm.shape[1]
    ngrp = k_hbm.shape[0] // _GRP
    d = wq_hbm.shape[0]
    bf16, f32 = jnp.bfloat16, jnp.float32
    rows = _GRP // nsplit

    def kv_copies(src, dst, sem, g, slot):
        return [
            pltpu.make_async_copy(
                src.at[pl.ds(pl.multiple_of(g * _GRP + i * rows, 16), rows), pl.ds(sk - win, win)],
                dst.at[slot, pl.ds(i * rows, rows)],
                sem.at[slot, i])
            for i in range(nsplit)
        ]

    def start(cs):
        for c in cs:
            c.start()

    def wait(cs):
        for c in cs:
            c.wait()

    c_x = pltpu.make_async_copy(x_hbm, x_v, sem_s.at[0])
    c_wq = pltpu.make_async_copy(wq_hbm, wq_v, sem_s.at[1])
    c_wo = pltpu.make_async_copy(wo_hbm, wo_v, sem_s.at[2])
    c_wr = pltpu.make_async_copy(wr_hbm, wr_v, sem_s.at[3])
    c_wg = pltpu.make_async_copy(wg_hbm, wg_v, sem_s.at[4])
    c_wu = pltpu.make_async_copy(wu_hbm, wu_v, sem_s.at[5])
    c_wd = pltpu.make_async_copy(wd_hbm, wd_v, sem_s.at[6])

    c_x.start()
    c_wq.start()
    start(kv_copies(k_hbm, k_v, sem_k, 0, 0))
    start(kv_copies(v_hbm, v_v, sem_v, 0, 0))
    c_wo.start()
    c_wr.start()
    for g in range(1, nbuf):
        start(kv_copies(k_hbm, k_v, sem_k, g, g))
        start(kv_copies(v_hbm, v_v, sem_v, g, g))

    row = lax.broadcasted_iota(jnp.int32, (8, _GRP), 0)
    col = lax.broadcasted_iota(jnp.int32, (8, _GRP), 1)
    diag = jnp.where(col < _DH, 0, 1) == row

    c_x.wait()
    x = x_v[0].astype(f32)
    xn = jnp.broadcast_to(_layernorm(x), (8, d)).astype(bf16)
    c_wq.wait()
    for g in range(ngrp):
        q = jnp.dot(xn, wq_v[:, g * _GRP:(g + 1) * _GRP], preferred_element_type=f32)
        q_v[g] = jnp.where(diag, q, 0.0)
    c_wo.wait()

    scale = _DH ** -0.5

    def body(g, acc):
        slot = lax.rem(g, nbuf)
        nxt = g + nbuf
        wait(kv_copies(k_hbm, k_v, sem_k, g, slot))
        s = jnp.dot(q_v[g].astype(bf16), k_v[slot], preferred_element_type=f32) * scale
        m = jnp.max(s, axis=-1, keepdims=True)
        p = jnp.exp(s - m)
        l = jnp.sum(p, axis=-1, keepdims=True)

        @pl.when(nxt < ngrp)
        def _():
            start(kv_copies(k_hbm, k_v, sem_k, nxt, slot))

        @pl.when(nxt == ngrp)
        def _():
            c_wg.start()
            c_wu.start()
            c_wd.start()

        wait(kv_copies(v_hbm, v_v, sem_v, g, slot))
        o = lax.dot_general(p.astype(bf16), v_v[slot], _NT, preferred_element_type=f32)

        @pl.when(nxt < ngrp)
        def _():
            start(kv_copies(v_hbm, v_v, sem_v, nxt, slot))

        o = jnp.where(diag, o / l, 0.0).astype(bf16)
        wo_blk = wo_v[pl.ds(pl.multiple_of(g * _GRP, _GRP), _GRP), :]
        return acc + jnp.dot(o, wo_blk, preferred_element_type=f32)

    acc = lax.fori_loop(0, ngrp, body, jnp.zeros((8, d), f32))
    h = x + jnp.sum(acc, axis=0, keepdims=True)
    hn = _layernorm(h)
    hb = jnp.broadcast_to(hn, (8, d)).astype(bf16)
    c_wr.wait()
    r = jnp.sum(hn * wr_v[...].astype(f32).reshape(1, d), axis=-1, keepdims=True)
    c_wg.wait()
    gate = jnp.dot(hb, wg_v[...], preferred_element_type=f32)
    c_wu.wait()
    up = jnp.dot(hb, wu_v[...], preferred_element_type=f32)
    act = (gate * jax.nn.sigmoid(gate) * up).astype(bf16)
    c_wd.wait()
    y = jnp.dot(act, wd_v[...], preferred_element_type=f32)[0:1]
    y = y * jax.nn.sigmoid(r)
    o_ref[0] = (h + (hn + (hn * 0.0 + y))).astype(o_ref.dtype)


def _run(A_x, A_k_cache, A_v_cache, A_wq, A_wo, B_w_r, B_w_gate, B_w_up, B_w_down,
         nbuf=3, nsplit=1):
    b, hkv, sk, dh = A_k_cache.shape
    d = A_x.shape[-1]
    f = B_w_gate.shape[1]
    assert (b, hkv, dh) == (1, _HQ, _DH) and A_x.shape == (1, 1, d)
    win = min(4096, max(256, sk // 4))
    kt = jnp.transpose(A_k_cache, (0, 1, 3, 2)).reshape(hkv * dh, sk)
    vt = jnp.transpose(A_v_cache, (0, 1, 3, 2)).reshape(hkv * dh, sk)
    bf16 = jnp.bfloat16
    any_spec = pl.BlockSpec(memory_space=pl.ANY)
    return pl.pallas_call(
        functools.partial(_kernel, win=win, nbuf=nbuf, nsplit=nsplit),
        in_specs=[any_spec] * 9,
        out_specs=pl.BlockSpec(memory_space=pltpu.VMEM),
        out_shape=jax.ShapeDtypeStruct(A_x.shape, A_x.dtype),
        scratch_shapes=[
            pltpu.VMEM((1, 1, d), bf16),
            pltpu.VMEM((d,), bf16),
            pltpu.VMEM((nbuf, _GRP, win), bf16),
            pltpu.VMEM((nbuf, _GRP, win), bf16),
            pltpu.VMEM((d, hkv * dh), bf16),
            pltpu.VMEM((hkv * dh, d), bf16),
            pltpu.VMEM((d, f), bf16),
            pltpu.VMEM((d, f), bf16),
            pltpu.VMEM((f, d), bf16),
            pltpu.VMEM((hkv // 2, 8, _GRP), jnp.float32),
            pltpu.SemaphoreType.DMA((7,)),
            pltpu.SemaphoreType.DMA((nbuf, nsplit)),
            pltpu.SemaphoreType.DMA((nbuf, nsplit)),
        ],
        compiler_params=pltpu.CompilerParams(vmem_limit_bytes=100 * 1024 * 1024),
    )(A_x, kt, vt, A_wq, A_wo, B_w_r, B_w_gate, B_w_up, B_w_down)


@jax.jit
def pallas_sequential_preLN__sliding_block_cached__moe_arch_mod__decode_kernel(
    A_x: jax.Array,
    A_k_cache: jax.Array,
    A_v_cache: jax.Array,
    A_wq: jax.Array,
    A_wo: jax.Array,
    B_x: jax.Array,
    B_w_r: jax.Array,
    B_w_gate: jax.Array,
    B_w_up: jax.Array,
    B_w_down: jax.Array,
):
    del B_x
    return _run(A_x, A_k_cache, A_v_cache, A_wq, A_wo, B_w_r, B_w_gate, B_w_up, B_w_down)
```
